```python
import os as _os
_os.environ.setdefault('JAX_PLATFORMS', 'cpu')
import jax
import jax.numpy as jnp

def _softmax(x, axis=-1):
    return jax.nn.softmax(x, axis=axis)

def _gelu(x):
    return jax.nn.gelu(x, approximate=True)

def _silu(x):
    return jax.nn.silu(x)

def _sigmoid(x):
    return jax.nn.sigmoid(x)

def _layernorm(x, axis=-1, eps=1e-05):
    m = jnp.mean(x, axis=axis, keepdims=True)
    v = jnp.var(x, axis=axis, keepdims=True)
    return (x - m) / jnp.sqrt(v + eps)

def _scatter_add(tgt, idx, src, axis=0):
    return tgt.at[idx].add(src)

def _segment_sum(src, seg, n):
    return jax.ops.segment_sum(src, seg, n)

class _Rng:

    def __init__(self, key):
        self._k = key

    def _next(self):
        self._k, sub = jax.random.split(self._k)
        return sub

    def normal(self, shape):
        return jax.random.normal(self._next(), shape, dtype=jnp.bfloat16)

    def randint(self, lo, hi, shape):
        return jax.random.randint(self._next(), shape, lo, hi, dtype=jnp.int32)

    def uniform(self, shape, lo=0.0, hi=1.0):
        return jax.random.uniform(self._next(), shape, jnp.bfloat16, lo, hi)

    def permutation(self, n):
        return jax.random.permutation(self._next(), n)
kernel_name = 'adaLN_cond__sliding_local_dilated__dense_activation_relu__prompt'

def setup_inputs():
    _rng = _Rng(jax.random.key(int.from_bytes(__import__("os").urandom(4), "little")))
    _w = lambda a: (lambda t: t.astype(jnp.bfloat16) if jnp.issubdtype(t.dtype, jnp.floating) else t)(jnp.asarray(a))

    def _A_setup():
        B, S, D = (1, 2048, 576)
        return {'x': _w((lambda *s: _rng.normal(s) * 0.05)(B, S, D)), 'wqkv': _w((lambda *s: _rng.normal(s) * 0.05)(D, 3 * D)), 'wo': _w((lambda *s: _rng.normal(s) * 0.05)(D, D))}
    _A_in = _A_setup()

    def _B_setup():
        B, S, D, Dff = (1, 2048, 576, 4608)
        return {'x': _w((lambda *s: _rng.normal(s) * 0.05)(B, S, D)), 'w1': _w((lambda *s: _rng.normal(s) * 0.05)(D, Dff)), 'w2': _w((lambda *s: _rng.normal(s) * 0.05)(Dff, D))}
    _B_in = _B_setup()
    return {'A_x': _A_in['x'], 'A_wqkv': _A_in['wqkv'], 'A_wo': _A_in['wo'], 'B_x': _B_in['x'], 'B_w1': _B_in['w1'], 'B_w2': _B_in['w2'], 'c': _w((lambda *s: _rng.normal(s) * 0.05)(1, 576) * 8.0), 'w_mod': _w((lambda *s: _rng.normal(s) * 0.05)(576, 6 * 576) * 576 ** (-0.5) * 8.0)}

def reference(A_x, A_wqkv, A_wo, B_x, B_w1, B_w2, c, w_mod):

    def _A_ref(x, wqkv, wo):
        B, S, D = x.shape
        H = 32
        Dh = D // H
        W, dil = (8, 2)
        qkv = (lambda x, *d: x.transpose(*d))((x @ wqkv).reshape(B, S, 3, H, Dh), 2, 0, 3, 1, 4)
        q, k, v = (qkv[0], qkv[1], qkv[2])
        scale = Dh ** (-0.5)
        pos = jnp.arange(S)
        off = jnp.arange(W) * dil
        idx = pos[:, None] - off[None, :]
        mask = idx >= 0
        idx_c = jnp.where(mask, idx, 0).reshape(-1)
        kg = k[:, :, idx_c, :].reshape(B, H, S, W, Dh)
        vg = v[:, :, idx_c, :].reshape(B, H, S, W, Dh)
        logits = jnp.einsum('bhsd,bhswd->bhsw', q, kg) * scale
        logits = jnp.where(mask[None, None, :, :], logits, -1000000000.0)
        attn = _softmax(logits, axis=-1)
        o = jnp.einsum('bhsw,bhswd->bhsd', attn, vg)
        return (lambda x, *d: x.transpose(*d))(o, 0, 2, 1, 3).reshape(B, S, D) @ wo

    def _B_ref(x, w1, w2):
        h = jnp.einsum('bsd,df->bsf', x, w1)
        zero = jnp.zeros_like(h)
        h = jnp.maximum(h, zero)
        return jnp.einsum('bsf,fd->bsd', h, w2)
    x = A_x
    mod = (_silu(c) @ w_mod).reshape(c.shape[0], 6, 1, -1)
    sa, ca, ga, sb, cb, gb = (mod[:, 0].copy(), mod[:, 1].copy(), mod[:, 2].copy(), mod[:, 3].copy(), mod[:, 4].copy(), mod[:, 5].copy())
    h = _layernorm(x, axis=-1) * (1 + ca) + sa
    x = x + ga * _A_ref(h, A_wqkv, A_wo)
    h = _layernorm(x, axis=-1) * (1 + cb) + sb
    x = x + gb * _B_ref(h, B_w1, B_w2)
    return x
```

```python
import functools
import jax
import jax.numpy as jnp
import jax.experimental.pallas as pl
import jax.experimental.pallas.tpu as pltpu

S, D, H, DH, W, DIL, DFF = 2048, 576, 32, 18, 8, 2, 4608
TILES = ((0, 128), (128, 256), (384, 512), (896, 1152))
NTL = len(TILES)
WC = 2304
NWC = DFF // WC
F32 = jnp.float32
BF16 = jnp.bfloat16
SX, SQKV, SMOD0, SMOD1, SWO, SW1, SW2, SOUT = 0, 5, 6, 7, 8, 9, 12, 15
NSEM = 20


def _ln_t(x):
    m = jnp.mean(x, axis=0, keepdims=True)
    xc = x - m
    v = jnp.mean(xc * xc, axis=0, keepdims=True)
    return xc * jax.lax.rsqrt(v + 1e-5)


def _kernel(c_ref, xt_hbm, wmod_hbm, wqkv_hbm, wo_hbm, w1_hbm, w2t_hbm, o_hbm,
            x_v, wmod_v, wqkv_v, wo_v, w1_v, w2t_v, wqkvt_v, wot_v, w1t_v,
            mod_ref, q_ref, kext_ref, vext_ref, oat_ref, x1_ref, h2_ref, acc_ref,
            out_v, stage_ref, wop_ref, sems):

    def cp_x(t):
        o, n = TILES[t]
        return pltpu.make_async_copy(xt_hbm.at[:, pl.ds(o, n)], x_v.at[:, pl.ds(o, n)], sems.at[SX + t])

    def cp_out(t):
        o, n = TILES[t]
        return pltpu.make_async_copy(out_v.at[:, pl.ds(o, n)], o_hbm.at[:, pl.ds(o, n)], sems.at[SOUT + t])

    cp_qkv = pltpu.make_async_copy(wqkv_hbm, wqkv_v, sems.at[SQKV])
    cp_mod0 = pltpu.make_async_copy(wmod_hbm.at[:, pl.ds(0, 2 * D)], wmod_v.at[:, pl.ds(0, 2 * D)],
                                    sems.at[SMOD0])
    cp_mod1 = pltpu.make_async_copy(wmod_hbm.at[:, pl.ds(2 * D, 4 * D)], wmod_v.at[:, pl.ds(2 * D, 4 * D)],
                                    sems.at[SMOD1])
    cp_wo = pltpu.make_async_copy(wo_hbm, wo_v, sems.at[SWO])

    def cp_w1(j):
        return pltpu.make_async_copy(w1_hbm.at[:, pl.ds(j * WC, WC)], w1_v.at[:, pl.ds(j * WC, WC)],
                                     sems.at[SW1 + j])

    def cp_w2(j):
        return pltpu.make_async_copy(w2t_hbm.at[:, pl.ds(j * WC, WC)], w2t_v.at[:, pl.ds(j * WC, WC)],
                                     sems.at[SW2 + j])

    def modv(j, n):
        m = mod_ref[j * D:(j + 1) * D, :]
        return m if n == 128 else jnp.concatenate([m] * (n // 128), axis=1)

    cp_qkv.start()
    cp_x(0).start()
    cp_mod0.start()
    cp_x(1).start()
    cp_wo.start()
    cp_mod1.start()
    for j in range(NWC):
        cp_w1(j).start()
        cp_w2(j).start()
        cp_x(2 + j).start()
    kext_ref[:, 0:128] = jnp.zeros((D, 128), BF16)
    vext_ref[:, 0:128] = jnp.zeros((D, 128), BF16)
    cp_qkv.wait()
    wt = wqkv_v[...].astype(F32).T
    for cb in range(5):
        n = 128 if cb < 4 else 64
        stage_ref[cb, :, 0:n] = wt[:, cb * 128:cb * 128 + n]
    for sec in range(3):
        for d in range(DH):
            for cb in range(5):
                n = 128 if cb < 4 else 64
                blk = stage_ref[cb, pl.ds(sec * D + d, H, stride=DH), :]
                wqkvt_v[sec * D + d * H: sec * D + (d + 1) * H, cb * 128:cb * 128 + n] = (
                    blk[:, 0:n].astype(BF16))
    c = c_ref[...].astype(F32)
    sc8 = jnp.broadcast_to((c * jax.nn.sigmoid(c)).astype(BF16), (8, D))
    cp_mod0.wait()
    modrow = jnp.dot(sc8, wmod_v[:, 0:2 * D], preferred_element_type=F32)
    mod_ref[0:2 * D, :] = jnp.broadcast_to(jnp.transpose(modrow)[:, 0:1], (2 * D, 128))

    def phase_a(t):
        o, n = TILES[t]
        cp_x(t).wait()
        x = x_v[:, o:o + n].astype(F32)
        h = (_ln_t(x) * (1.0 + modv(1, n)) + modv(0, n)).astype(BF16)
        qkv = jnp.dot(wqkvt_v[...], h, preferred_element_type=F32)
        q_ref[:, o:o + n] = qkv[0:D]
        kext_ref[:, 128 + o:128 + o + n] = qkv[D:2 * D].astype(BF16)
        vext_ref[:, 128 + o:128 + o + n] = qkv[2 * D:3 * D].astype(BF16)

    def attn(off, n):
        spos = off + jax.lax.broadcasted_iota(jnp.int32, (H, n), 1)

        def sh(a, w):
            return a[:, 128 - DIL * w:128 + n - DIL * w].astype(F32)
        logits = [None] * W
        for d in range(DH):
            q = q_ref[d * H:(d + 1) * H, pl.ds(off, n)]
            kwin = kext_ref[d * H:(d + 1) * H, pl.ds(off, n + 128)]
            for w in range(W):
                p = q * sh(kwin, w)
                logits[w] = p if logits[w] is None else logits[w] + p
        logits = [jnp.where(spos >= DIL * w, logits[w] * DH ** -0.5, -1e9) for w in range(W)]
        m = logits[0]
        for w in range(1, W):
            m = jnp.maximum(m, logits[w])
        es = [jnp.exp(l - m) for l in logits]
        den = es[0]
        for w in range(1, W):
            den = den + es[w]
        inv = 1.0 / den
        aw = [e * inv for e in es]
        for d in range(DH):
            vwin = vext_ref[d * H:(d + 1) * H, pl.ds(off, n + 128)]
            o = None
            for w in range(W):
                t_ = aw[w] * sh(vwin, w)
                o = t_ if o is None else o + t_
            oat_ref[d * H:(d + 1) * H, pl.ds(off, n)] = o.astype(BF16)

    def phase_c(t):
        o, n = TILES[t]
        att = jnp.dot(wot_v[...], oat_ref[:, o:o + n], preferred_element_type=F32)
        x1 = x_v[:, o:o + n].astype(F32) + modv(2, n) * att
        x1_ref[:, o:o + n] = x1
        h2_ref[:, o:o + n] = (_ln_t(x1) * (1.0 + modv(4, n)) + modv(3, n)).astype(BF16)

    def ffn_chunk(t, foff, fc, first):
        o, n = TILES[t]
        a = jnp.dot(w1t_v[pl.ds(foff, fc), :], h2_ref[:, o:o + n], preferred_element_type=F32)
        a = jnp.maximum(a, 0.0).astype(BF16)
        y = jnp.dot(w2t_v[:, pl.ds(foff, fc)], a, preferred_element_type=F32)
        if first:
            acc_ref[:, 0:n] = y
        else:
            acc_ref[:, 0:n] += y

    def finish(t):
        o, n = TILES[t]
        out_v[:, o:o + n] = (x1_ref[:, o:o + n] + modv(5, n) * acc_ref[:, 0:n]).astype(BF16)
        cp_out(t).start()

    phase_a(0)
    attn(0, 128)
    cp_wo.wait()
    wof = wo_v[...].astype(F32)
    for cb in range(5):
        n = 128 if cb < 4 else 64
        stage_ref[cb, 0:D, 0:n] = wof[:, cb * 128:cb * 128 + n]
    for d in range(DH):
        for cb in range(5):
            n = 128 if cb < 4 else 64
            blk = stage_ref[cb, pl.ds(d, H, stride=DH), :]
            wop_ref[d * H:(d + 1) * H, cb * 128:cb * 128 + n] = blk[:, 0:n]
    wot_v[...] = wop_ref[...].T.astype(BF16)
    cp_mod1.wait()
    modrow = jnp.dot(sc8, wmod_v[:, 2 * D:6 * D], preferred_element_type=F32)
    mod_ref[2 * D:6 * D, :] = jnp.broadcast_to(jnp.transpose(modrow)[:, 0:1], (4 * D, 128))
    phase_c(0)

    phase_a(1)
    for j in range(NWC):
        cp_w1(j).wait()
        cp_w2(j).wait()
        w1t_v[j * WC:(j + 1) * WC, :] = w1_v[:, j * WC:(j + 1) * WC].T
        ffn_chunk(0, j * WC, WC, j == 0)
        attn(TILES[1][0] + j * 128, 128)
    finish(0)
    phase_c(1)

    for t in range(2, NTL):
        phase_a(t)
        nc = TILES[t][1] // 128
        fc = DFF // nc
        acc_ref[...] = jnp.zeros_like(acc_ref)

        def body(f, carry, t=t, fc=fc):
            ffn_chunk(t - 1, pl.multiple_of(f * fc, fc), fc, False)
            attn(pl.multiple_of(TILES[t][0] + f * 128, 128), 128)
            return carry
        jax.lax.fori_loop(0, nc, body, 0)
        finish(t - 1)
        phase_c(t)

    acc_ref[...] = jnp.zeros_like(acc_ref)

    def body(f, carry):
        ffn_chunk(NTL - 1, pl.multiple_of(f * 512, 512), 512, False)
        return carry
    jax.lax.fori_loop(0, DFF // 512, body, 0)
    finish(NTL - 1)
    for t in range(NTL):
        cp_out(t).wait()


@jax.jit
def pallas_adaLN_cond__sliding_local_dilated__dense_activation_relu__prompt_kernel(
    A_x, A_wqkv, A_wo, B_x, B_w1, B_w2, c, w_mod):
    xt = A_x.reshape(S, D).T
    w2t = B_w2.T
    hbm = pl.BlockSpec(memory_space=pl.ANY)
    out = pl.pallas_call(
        _kernel,
        in_specs=[pl.BlockSpec(memory_space=pltpu.VMEM), hbm, hbm, hbm, hbm, hbm, hbm],
        out_specs=hbm,
        out_shape=jax.ShapeDtypeStruct((D, S), BF16),
        scratch_shapes=[
            pltpu.VMEM((D, S), BF16),
            pltpu.VMEM((D, 6 * D), BF16), pltpu.VMEM((D, 3 * D), BF16), pltpu.VMEM((D, D), BF16),
            pltpu.VMEM((D, DFF), BF16), pltpu.VMEM((D, DFF), BF16),
            pltpu.VMEM((3 * D, D), BF16), pltpu.VMEM((D, D), BF16), pltpu.VMEM((DFF, D), BF16),
            pltpu.VMEM((6 * D, 128), F32),
            pltpu.VMEM((D, S), F32),
            pltpu.VMEM((D, S + 128), BF16),
            pltpu.VMEM((D, S + 128), BF16),
            pltpu.VMEM((D, S), BF16),
            pltpu.VMEM((D, S), F32),
            pltpu.VMEM((D, S), BF16),
            pltpu.VMEM((D, 1152), F32),
            pltpu.VMEM((D, S), BF16),
            pltpu.VMEM((5, 3 * D, 128), F32), pltpu.VMEM((D, D), F32),
            pltpu.SemaphoreType.DMA((NSEM,)),
        ],
        compiler_params=pltpu.CompilerParams(vmem_limit_bytes=100 * 1024 * 1024),
    )(c, xt, w_mod, A_wqkv, A_wo, B_w1, w2t)
    return out.T.reshape(1, S, D)
```

```python
import jax
import jax.numpy as jnp
import jax.experimental.pallas as pl
import jax.experimental.pallas.tpu as pltpu

S, D, H, DH, W, DIL, DFF = 2048, 576, 32, 18, 8, 2, 4608
TILES = ((0, 128), (128, 256), (384, 512), (896, 1152))
NTL = len(TILES)
WC = 2304
NWC = DFF // WC
F32 = jnp.float32
BF16 = jnp.bfloat16
SX, SQKV, SMOD0, SMOD1, SWO, SW1, SW2, SOUT = 0, 5, 6, 7, 8, 9, 12, 15
NSEM = 20


def _ln_t(x):
    m = jnp.mean(x, axis=0, keepdims=True)
    xc = x - m
    v = jnp.mean(xc * xc, axis=0, keepdims=True)
    return xc * jax.lax.rsqrt(v + 1e-5)


def _kernel(c_ref, xt_hbm, wmod_hbm, wqkv_hbm, wo_hbm, w1_hbm, w2t_hbm, o_hbm,
            x_v, wmod_v, wqkv_v, wo_v, w1_v, w2t_v, wqkvt_v, wot_v, w1t_v,
            mod_ref, q_ref, kext_ref, vext_ref, oat_ref, x1_ref, h2_ref, acc_ref,
            out_v, stage_ref, wop_ref, sems):

    def cp_x(t):
        o, n = TILES[t]
        return pltpu.make_async_copy(xt_hbm.at[:, pl.ds(o, n)], x_v.at[:, pl.ds(o, n)], sems.at[SX + t])

    def cp_out(t):
        o, n = TILES[t]
        return pltpu.make_async_copy(out_v.at[:, pl.ds(o, n)], o_hbm.at[:, pl.ds(o, n)], sems.at[SOUT + t])

    cp_qkv = pltpu.make_async_copy(wqkv_hbm, wqkv_v, sems.at[SQKV])
    cp_mod0 = pltpu.make_async_copy(wmod_hbm.at[:, pl.ds(0, 2 * D)], wmod_v.at[:, pl.ds(0, 2 * D)],
                                    sems.at[SMOD0])
    cp_mod1 = pltpu.make_async_copy(wmod_hbm.at[:, pl.ds(2 * D, 4 * D)], wmod_v.at[:, pl.ds(2 * D, 4 * D)],
                                    sems.at[SMOD1])
    cp_wo = pltpu.make_async_copy(wo_hbm, wo_v, sems.at[SWO])

    def cp_w1(j):
        return pltpu.make_async_copy(w1_hbm.at[:, pl.ds(j * WC, WC)], w1_v.at[:, pl.ds(j * WC, WC)],
                                     sems.at[SW1 + j])

    def cp_w2(j):
        return pltpu.make_async_copy(w2t_hbm.at[:, pl.ds(j * WC, WC)], w2t_v.at[:, pl.ds(j * WC, WC)],
                                     sems.at[SW2 + j])

    def modv(j, n):
        m = mod_ref[j * D:(j + 1) * D, :]
        return m if n == 128 else jnp.concatenate([m] * (n // 128), axis=1)

    cp_mod0.start()
    cp_x(0).start()
    cp_qkv.start()
    cp_x(1).start()
    cp_wo.start()
    cp_mod1.start()
    cp_x(2).start()
    cp_x(3).start()
    for j in range(NWC):
        cp_w1(j).start()
        cp_w2(j).start()
    kext_ref[:, 0:128] = jnp.zeros((D, 128), BF16)
    vext_ref[:, 0:128] = jnp.zeros((D, 128), BF16)
    c = c_ref[...].astype(F32)
    sc8 = jnp.broadcast_to((c * jax.nn.sigmoid(c)).astype(BF16), (8, D))
    cp_mod0.wait()
    modrow = jnp.dot(sc8, wmod_v[:, 0:2 * D], preferred_element_type=F32)
    mod_ref[0:2 * D, :] = jnp.broadcast_to(jnp.transpose(modrow)[:, 0:1], (2 * D, 128))
    cp_qkv.wait()
    wt = wqkv_v[...].astype(F32).T
    for cb in range(5):
        n = 128 if cb < 4 else 64
        stage_ref[cb, :, 0:n] = wt[:, cb * 128:cb * 128 + n]
    for sec in range(3):
        for d in range(DH):
            for cb in range(5):
                n = 128 if cb < 4 else 64
                blk = stage_ref[cb, pl.ds(sec * D + d, H, stride=DH), :]
                wqkvt_v[sec * D + d * H: sec * D + (d + 1) * H, cb * 128:cb * 128 + n] = (
                    blk[:, 0:n].astype(BF16))

    def phase_a_rng(o, n):
        x = x_v[:, pl.ds(o, n)].astype(F32)
        h = (_ln_t(x) * (1.0 + modv(1, n)) + modv(0, n)).astype(BF16)
        qkv = jnp.dot(wqkvt_v[...], h, preferred_element_type=F32)
        q_ref[:, pl.ds(o, n)] = qkv[0:D]
        kext_ref[:, pl.ds(128 + o, n)] = qkv[D:2 * D].astype(BF16)
        vext_ref[:, pl.ds(128 + o, n)] = qkv[2 * D:3 * D].astype(BF16)

    def phase_a(t):
        phase_a_rng(*TILES[t])

    def attn(off, n):
        spos = off + jax.lax.broadcasted_iota(jnp.int32, (H, n), 1)

        def sh(a, w):
            return a[:, 128 - DIL * w:128 + n - DIL * w].astype(F32)
        logits = [None] * W
        for d in range(DH):
            q = q_ref[d * H:(d + 1) * H, pl.ds(off, n)]
            kwin = kext_ref[d * H:(d + 1) * H, pl.ds(off, n + 128)]
            for w in range(W):
                p = q * sh(kwin, w)
                logits[w] = p if logits[w] is None else logits[w] + p
        logits = [jnp.where(spos >= DIL * w, logits[w] * DH ** -0.5, -1e9) for w in range(W)]
        m = logits[0]
        for w in range(1, W):
            m = jnp.maximum(m, logits[w])
        es = [jnp.exp(l - m) for l in logits]
        den = es[0]
        for w in range(1, W):
            den = den + es[w]
        inv = 1.0 / den
        aw = [e * inv for e in es]
        for d in range(DH):
            vwin = vext_ref[d * H:(d + 1) * H, pl.ds(off, n + 128)]
            o = None
            for w in range(W):
                t_ = aw[w] * sh(vwin, w)
                o = t_ if o is None else o + t_
            oat_ref[d * H:(d + 1) * H, pl.ds(off, n)] = o.astype(BF16)

    def phase_c(t):
        o, n = TILES[t]
        att = jnp.dot(wot_v[...], oat_ref[:, o:o + n], preferred_element_type=F32)
        x1 = x_v[:, o:o + n].astype(F32) + modv(2, n) * att
        x1_ref[:, o:o + n] = x1
        h2_ref[:, o:o + n] = (_ln_t(x1) * (1.0 + modv(4, n)) + modv(3, n)).astype(BF16)

    def ffn_chunk(t, foff, fc, first):
        o, n = TILES[t]
        a = jnp.dot(w1t_v[pl.ds(foff, fc), :], h2_ref[:, o:o + n], preferred_element_type=F32)
        a = jnp.maximum(a, 0.0).astype(BF16)
        y = jnp.dot(w2t_v[:, pl.ds(foff, fc)], a, preferred_element_type=F32)
        if first:
            acc_ref[:, 0:n] = y
        else:
            acc_ref[:, 0:n] += y

    def finish(t):
        o, n = TILES[t]
        out_v[:, o:o + n] = (x1_ref[:, o:o + n] + modv(5, n) * acc_ref[:, 0:n]).astype(BF16)
        cp_out(t).start()

    cp_x(0).wait()
    phase_a(0)
    cp_x(1).wait()
    cp_wo.wait()
    cp_mod1.wait()
    attn(0, 128)
    wof = wo_v[...].astype(F32)
    for cb in range(5):
        n = 128 if cb < 4 else 64
        stage_ref[cb, 0:D, 0:n] = wof[:, cb * 128:cb * 128 + n]
    for d in range(DH):
        for cb in range(5):
            n = 128 if cb < 4 else 64
            blk = stage_ref[cb, pl.ds(d, H, stride=DH), :]
            wop_ref[d * H:(d + 1) * H, cb * 128:cb * 128 + n] = blk[:, 0:n]
    wot_v[...] = wop_ref[...].T.astype(BF16)
    modrow = jnp.dot(sc8, wmod_v[:, 2 * D:6 * D], preferred_element_type=F32)
    mod_ref[2 * D:6 * D, :] = jnp.broadcast_to(jnp.transpose(modrow)[:, 0:1], (4 * D, 128))
    phase_c(0)

    cp_x(2).wait()
    cp_x(3).wait()
    def body_a(f, carry):
        phase_a_rng(pl.multiple_of(128 + f * 384, 128), 384)
        return carry
    jax.lax.fori_loop(0, 5, body_a, 0)
    for j in range(NWC):
        cp_w1(j).wait()
        cp_w2(j).wait()
        w1t_v[j * WC:(j + 1) * WC, :] = w1_v[:, j * WC:(j + 1) * WC].T
        ffn_chunk(0, j * WC, WC, j == 0)
        attn(TILES[1][0] + j * 128, 128)
    finish(0)
    phase_c(1)

    for t in range(2, NTL):
        nc = TILES[t][1] // 128
        fc = DFF // nc
        acc_ref[...] = jnp.zeros_like(acc_ref)

        def body(f, carry, t=t, fc=fc):
            ffn_chunk(t - 1, pl.multiple_of(f * fc, fc), fc, False)
            attn(pl.multiple_of(TILES[t][0] + f * 128, 128), 128)
            return carry
        jax.lax.fori_loop(0, nc, body, 0)
        finish(t - 1)
        phase_c(t)

    acc_ref[...] = jnp.zeros_like(acc_ref)

    def body(f, carry):
        ffn_chunk(NTL - 1, pl.multiple_of(f * 512, 512), 512, False)
        return carry
    jax.lax.fori_loop(0, DFF // 512, body, 0)
    finish(NTL - 1)
    for t in range(NTL):
        cp_out(t).wait()


@jax.jit
def pallas_adaLN_cond__sliding_local_dilated__dense_activation_relu__prompt_kernel(
    A_x, A_wqkv, A_wo, B_x, B_w1, B_w2, c, w_mod):
    xt = A_x.reshape(S, D).T
    w2t = B_w2.T
    hbm = pl.BlockSpec(memory_space=pl.ANY)
    out = pl.pallas_call(
        _kernel,
        in_specs=[pl.BlockSpec(memory_space=pltpu.VMEM), hbm, hbm, hbm, hbm, hbm, hbm],
        out_specs=hbm,
        out_shape=jax.ShapeDtypeStruct((D, S), BF16),
        scratch_shapes=[
            pltpu.VMEM((D, S), BF16),
            pltpu.VMEM((D, 6 * D), BF16), pltpu.VMEM((D, 3 * D), BF16), pltpu.VMEM((D, D), BF16),
            pltpu.VMEM((D, DFF), BF16), pltpu.VMEM((D, DFF), BF16),
            pltpu.VMEM((3 * D, D), BF16), pltpu.VMEM((D, D), BF16), pltpu.VMEM((DFF, D), BF16),
            pltpu.VMEM((6 * D, 128), F32),
            pltpu.VMEM((D, S), F32),
            pltpu.VMEM((D, S + 128), BF16),
            pltpu.VMEM((D, S + 128), BF16),
            pltpu.VMEM((D, S), BF16),
            pltpu.VMEM((D, S), F32),
            pltpu.VMEM((D, S), BF16),
            pltpu.VMEM((D, 1152), F32),
            pltpu.VMEM((D, S), BF16),
            pltpu.VMEM((5, 3 * D, 128), F32), pltpu.VMEM((D, D), F32),
            pltpu.SemaphoreType.DMA((NSEM,)),
        ],
        compiler_params=pltpu.CompilerParams(vmem_limit_bytes=100 * 1024 * 1024),
    )(c, xt, w_mod, A_wqkv, A_wo, B_w1, w2t)
    return out.T.reshape(1, S, D)
```
